```python
import os as _os
_os.environ.setdefault("JAX_PLATFORMS", "cpu")
import jax
import jax.numpy as jnp

def _softmax(x, axis=-1):
    return jax.nn.softmax(x, axis=axis)
def _gelu(x):
    return jax.nn.gelu(x, approximate=True)
def _silu(x):
    return jax.nn.silu(x)
def _sigmoid(x):
    return jax.nn.sigmoid(x)
def _layernorm(x, axis=-1, eps=1e-5):
    m = jnp.mean(x, axis=axis, keepdims=True)
    v = jnp.var(x, axis=axis, keepdims=True)
    return (x - m) / jnp.sqrt(v + eps)
def _scatter_add(tgt, idx, src, axis=0):
    return tgt.at[idx].add(src)
def _segment_sum(src, seg, n):
    return jax.ops.segment_sum(src, seg, n)
class _Rng:
    def __init__(self, key):
        self._k = key
    def _next(self):
        self._k, sub = jax.random.split(self._k)
        return sub
    def normal(self, shape):
        return jax.random.normal(self._next(), shape, dtype=jnp.bfloat16)
    def randint(self, lo, hi, shape):
        return jax.random.randint(self._next(), shape, lo, hi, dtype=jnp.int32)
    def uniform(self, shape, lo=0.0, hi=1.0):
        return jax.random.uniform(self._next(), shape, jnp.bfloat16, lo, hi)
    def permutation(self, n):
        return jax.random.permutation(self._next(), n)


kernel_name = 'standalone__fft_conv__vision'

def setup_inputs():
    _rng = _Rng(jax.random.key(int.from_bytes(__import__("os").urandom(4), "little")))
    _w = (lambda a: (lambda t: t.astype(jnp.bfloat16) if jnp.issubdtype(t.dtype, jnp.floating) else t)(jnp.asarray(a)))
    H = W = 224
    C = 96
    K = 3
    return {
        "x": _w((lambda *s: _rng.normal(s) * 0.05)(1, H, W, C)),
        "w": _w((lambda *s: _rng.normal(s) * 0.05)(K, K, C, C)),
    }

def reference(x, w):
    B, H, W, C = x.shape
    K = w.shape[0]
    wp = jnp.pad(w, ((0, H - K), (0, W - K), (0, 0), (0, 0)))
    Xf = (lambda x, axes=(-2,-1): jnp.fft.rfft2(x.astype(jnp.float32), axes=axes))(x, axes=(1, 2))
    Wf = (lambda x, axes=(-2,-1): jnp.fft.rfft2(x.astype(jnp.float32), axes=axes))(wp, axes=(0, 1))
    Yf = jnp.einsum('bhwi,hwio->bhwo', Xf, Wf)
    y = (lambda x, s, axes=(-2,-1): jnp.fft.irfft2(x, s=s, axes=axes).astype(jnp.bfloat16))(Yf, (H, W), axes=(1, 2))
    return y
```

```python
import functools
import numpy as np
import jax, jax.numpy as jnp
from jax import lax
from jax.experimental import pallas as pl
from jax.experimental.pallas import tpu as pltpu

H = W = 224; C = 96
PA, PB = 2.0 / 3.0, 1.5
f32 = jnp.float32; bf16 = jnp.bfloat16; u32 = jnp.uint32
XF0 = H + 2

def g_matrix():
    pts = [0.0, PA, -PA, PB, -PB]
    G = []
    for j, p in enumerate(pts):
        f = 1.0
        for k, q in enumerate(pts):
            if k != j: f *= (p - q)
        G.append([1.0 / f, p / f, p * p / f])
    G.append([0.0, 0.0, 1.0])
    return G

def kernel(x_hbm, w_hbm, y_hbm, big, xb1, yb0, yb1, wraw, u_ref, ul_ref, su, ltu, in_sems, out_sem, *,
           T, chunks, thr, MC, corder, sched, outmode, wtr):
    NT = H // 4
    NIT = NT // T
    R = 16
    assert (4 * T) % R == 0
    NS = 4
    assert T % NS == 0
    D0 = XF0 + R
    DUM = D0 + 12 * NS
    a, b = PA, PB
    a2, b2 = a * a, b * b
    c = a2 + b2

    def in_copies(k):
        lo, hi = chunks[k]
        cps = []
        if k == 0:
            cps += [pltpu.make_async_copy(x_hbm.at[pl.ds(H - 2, 2), :, pl.ds(0, 128)], big.at[pl.ds(0, 2)], in_sems.at[k]),
                    pltpu.make_async_copy(x_hbm.at[pl.ds(H - 2, 2), :, pl.ds(128, 96)], xb1.at[pl.ds(0, 2)], in_sems.at[k])]
        cps += [pltpu.make_async_copy(x_hbm.at[pl.ds(lo, hi - lo), :, pl.ds(128, 96)], xb1.at[pl.ds(lo + 2, hi - lo)], in_sems.at[k]),
                pltpu.make_async_copy(x_hbm.at[pl.ds(lo, hi - lo), :, pl.ds(0, 128)], big.at[pl.ds(lo + 2, hi - lo)], in_sems.at[k])]
        return cps

    def out_copies(lo, n):
        return [pltpu.make_async_copy(yb0.at[pl.ds(lo, n)], y_hbm.at[pl.ds(lo, n), :, pl.ds(0, 128)], out_sem),
                pltpu.make_async_copy(yb1.at[pl.ds(lo, n)], y_hbm.at[pl.ds(lo, n), :, pl.ds(128, 96)], out_sem)]

    wcp = pltpu.make_async_copy(w_hbm, wraw, in_sems.at[len(chunks)])
    for cp in in_copies(0): cp.start()
    wcp.start()
    for k in range(1, len(chunks)):
        for cp in in_copies(k): cp.start()

    lane = lax.broadcasted_iota(jnp.int32, (8, 128), 1)
    m126 = lane >= 126; m127 = lane >= 127

    bigu = big.bitcast(u32); xb1u = xb1.bitcast(u32)
    uu = u_ref.bitcast(u32); ulu = ul_ref.bitcast(u32)

    def wprep():
        G = g_matrix()
        if wtr == "mxu":
            eye = (lax.broadcasted_iota(jnp.int32, (96, 96), 0) == lax.broadcasted_iota(jnp.int32, (96, 96), 1)).astype(bf16)
            tr = lambda m: lax.dot_general(eye, m.astype(bf16), (((1,), (1,)), ((), ())), preferred_element_type=f32).astype(bf16)
        else:
            tr = lambda m: m.astype(bf16).astype(f32).T.astype(bf16)
        def comb(j, kw, lo, hi):
            acc = None
            for r in range(3):
                if G[j][r] == 0.0: continue
                t = wraw[2 - r, kw, lo:hi, :].astype(f32) * G[j][r]
                acc = t if acc is None else acc + t
            return acc
        for j in range(6):
            u_ref[j, 0] = tr(jnp.concatenate([comb(j, 1, 0, 96), comb(j, 2, 0, 32)], axis=0))
            u_ref[j, 1] = tr(jnp.concatenate([comb(j, 2, 32, 96), comb(j, 0, 0, 64)], axis=0))
        z = jnp.zeros((32, 96), f32)
        t0, t1, t2 = [wraw[2 - r, 0, 64:96, :].astype(f32) for r in range(3)]
        ul_ref[0:96, :] = tr(jnp.concatenate([t0, t1, t2, z], axis=0))
        ul_ref[96:192, :] = tr(jnp.concatenate([z, t0, t1, t2], axis=0))

    def fix(row, ring):
        v = xb1u[row]
        bigu[XF0 + ring] = jnp.concatenate([v, v[:, 64:96]], axis=1)

    def dslab(slot, n, j):
        return D0 + (slot * 2 + n) * 6 + j

    def trans(tile, slot, vrs):
        r0 = tile * 4
        idx = [[r0 + k for k in range(6)], [XF0 + ((r0 + k) & (R - 1)) for k in range(6)]]
        for vr in vrs:
            rows = pl.ds(vr * 16, 16)
            for n in range(2):
                d = [big[idx[n][k], rows, :].astype(f32) for k in range(6)]
                if vr >= 4:
                    for k in range(6):
                        ltu[slot, n, pl.ds(k * 16 + (vr - 4) * 8, 8), :] = bigu[idx[n][k], pl.ds(vr * 8, 8), :]
                t = a2 * d[2]
                E1 = d[4] - b2 * d[2]; O1 = a * d[3] - b * d[1]
                E2 = d[4] - t; O2 = b * d[3] - a * d[1]
                D = [d[0] + E1 - t, E1 + O1, E1 - O1, E2 + O2, E2 - O2, d[1] - c * d[3] + d[5]]
                for j in range(6):
                    big[dslab(slot, n, j), rows, :] = D[j].astype(bf16)

    def rolls(slot, js):
        for j in js:
            for vr in range(6):
                v0 = bigu[dslab(slot, 0, j), pl.ds(vr * 8, 8), :]
                v1 = bigu[dslab(slot, 1, j), pl.ds(vr * 8, 8), :]
                s10 = pltpu.roll(jnp.where(m127, v1, v0), 1, 1)
                s20 = pltpu.roll(jnp.where(m126, v1, v0), 2, 1)
                v1p = jnp.where(m126, v0, v1)
                s11 = pltpu.roll(v1p, 1, 1)
                s21 = pltpu.roll(v1p, 2, 1)
                su[slot, 0, j, pl.ds(vr * 8, 8), :] = s10
                su[slot, 1, j, pl.ds(vr * 8, 8), :] = s11
                su[slot, 0, j, pl.ds(48 + vr * 8, 8), :] = s20
                su[slot, 1, j, pl.ds(48 + vr * 8, 8), :] = s21

    def dot(l, r):
        return jnp.dot(pltpu.bitcast(l, bf16), pltpu.bitcast(r, bf16), preferred_element_type=f32)

    def cons(tile, slot, part):
        r0 = tile * 4
        n, mc = part // (96 // MC), part % (96 // MC)
        mr = pl.ds(mc * MC // 2, MC // 2)
        def mm(j):
            k1 = jnp.concatenate([su[slot, n, j, pl.ds(64, 32), :], bigu[dslab(slot, n, j), pl.ds(0, 32), :]], axis=0)
            return dot(uu[j, 0, mr, :], su[slot, n, j, pl.ds(0, 64), :]) + dot(uu[j, 1, mr, :], k1)
        def ll(p, h):
            return dot(ulu[pl.ds(48 * h + mc * MC // 2, MC // 2), :], ltu[slot, n, pl.ds(32 * p, 64), :])
        if corder == 0:
            m1 = mm(1); m2 = mm(2)
            s12 = m1 + m2; d12 = m1 - m2
            m3 = mm(3); m4 = mm(4)
            s34 = m3 + m4; d34 = m3 - m4
            y = [s12 + s34, a * d12 + b * d34, a2 * s12 + b2 * s34, (a2 * a) * d12 + (b2 * b) * d34]
            m0 = mm(0); m5 = mm(5)
            ys = [y[0] + m0 + ll(0, 0), y[1] + ll(0, 1), y[2] + ll(1, 0), y[3] + m5 + ll(1, 1)]
        else:
            y = [ll(0, 0), ll(0, 1), ll(1, 0), ll(1, 1)]
            m0 = mm(0); m5 = mm(5)
            y[0] = y[0] + m0; y[3] = y[3] + m5
            m1 = mm(1); m2 = mm(2)
            s12 = m1 + m2; d12 = m1 - m2
            y = [y[0] + s12, y[1] + a * d12, y[2] + a2 * s12, y[3] + (a2 * a) * d12]
            m3 = mm(3); m4 = mm(4)
            s34 = m3 + m4; d34 = m3 - m4
            ys = [y[0] + s34, y[1] + b * d34, y[2] + b2 * s34, y[3] + (b2 * b) * d34]
        for q in range(4):
            if n == 0:
                yb0[r0 + q, pl.ds(mc * MC, MC), :] = ys[q].astype(bf16)
            else:
                yb1[r0 + q, pl.ds(mc * MC, MC), pl.ds(0, 128)] = ys[q].astype(bf16)
        if thr == "early":
            bigu[DUM, pl.ds(0, 8), :] = pltpu.bitcast(s12[0:8], u32)
        elif thr == "late":
            bigu[DUM, pl.ds(0, 8), :] = pltpu.bitcast(ys[3][MC - 8:MC], u32)

    jorder = (1, 2, 3, 4, 0, 5) if corder == 0 else (0, 5, 1, 2, 3, 4)
    zero = pl.program_id(0)

    for cp in in_copies(0): cp.wait()
    for r in range(6):
        fix(r, r)
    trans(zero, 0, range(6))
    wcp.wait()
    for cp in in_copies(1): cp.wait()
    for r in range(6, 10):
        fix(r, r)
    rolls(0, jorder)
    wprep()
    trans(zero + 1, 1, range(6))
    for r in range(10, 14):
        fix(r, r)

    def wrap(v):
        return jnp.where(v >= NT, v - NT, v)

    NP = 2 * (96 // MC)
    def body(it, carry):
        for k in range(2, len(chunks)):
            need_it = next(i for i in range(NIT) if min(((i + 1) * T + 3) * 4 + 2 - 2, H) > chunks[k][0])
            @pl.when(it == need_it)
            def _():
                for cp in in_copies(k): cp.wait()
        for t in range(T):
            cur = it * T + t
            n2 = wrap(cur + 2); n3 = wrap(cur + 3)
            s0 = t % NS; s1 = (t + 1) % NS; s2 = (t + 2) % NS
            def dofix():
                for k in range(2, 6):
                    fix(n3 * 4 + k, ((t + 3) * 4 + k) % R)
            if sched == 0 and NP == 4:
                rolls(s1, jorder[0:2]); trans(n2, s2, (0, 1)); cons(cur, s0, 0)
                rolls(s1, jorder[2:4]); trans(n2, s2, (2, 3)); cons(cur, s0, 1)
                rolls(s1, jorder[4:6]); trans(n2, s2, (4, 5)); cons(cur, s0, 2)
                dofix(); cons(cur, s0, 3)
            elif sched == 0 and NP == 6:
                for p in range(6):
                    rolls(s1, jorder[p:p + 1]); trans(n2, s2, (p,)); cons(cur, s0, p)
                dofix()
            elif sched == 0 and NP == 2:
                rolls(s1, jorder[0:3]); trans(n2, s2, (0, 1, 2)); cons(cur, s0, 0)
                rolls(s1, jorder[3:6]); trans(n2, s2, (3, 4, 5)); dofix(); cons(cur, s0, 1)
            elif sched == 1:
                for p in range(NP): cons(cur, s0, p)
                rolls(s1, jorder); trans(n2, s2, range(6)); dofix()
            if outmode == "tile":
                for cp in out_copies(cur * 4, 4): cp.start()
            if outmode.startswith("ltile"):
                @pl.when(it > int(outmode[5:]))
                def _():
                    for cp in out_copies(cur * 4, 4): cp.start()
        if outmode == "iter":
            for cp in out_copies(it * T * 4, T * 4): cp.start()
        if outmode.startswith("ltile"):
            osi = int(outmode[5:])
            @pl.when(it == osi)
            def _():
                for cp in out_copies(0, (osi + 1) * T * 4): cp.start()
        if outmode.startswith("late"):
            osi = int(outmode[4:])
            @pl.when(it == osi)
            def _():
                for cp in out_copies(0, (osi + 1) * T * 4): cp.start()
            @pl.when(it > osi)
            def _():
                for cp in out_copies(it * T * 4, T * 4): cp.start()
        return carry
    lax.fori_loop(0, NIT, body, 0)
    for cp in out_copies(0, H): cp.wait()

@functools.partial(jax.jit, static_argnames=("T", "chunks", "thr", "MC", "corder", "sched", "outmode", "wtr"))
def conv(x, w, T=4, chunks=((0, 4), (4, 12), (12, 28), (28, 60), (60, 124), (124, 224)), thr="late", MC=48, corder=0, sched=0, outmode="ltile4", wtr="mxu"):
    xt = jnp.transpose(x[0], (0, 2, 1))
    NS = 4
    yt = pl.pallas_call(
        functools.partial(kernel, T=T, chunks=chunks, thr=thr, MC=MC, corder=corder, sched=sched, outmode=outmode, wtr=wtr),
        grid=(1,),
        in_specs=[pl.BlockSpec(memory_space=pl.ANY), pl.BlockSpec(memory_space=pl.ANY)],
        out_specs=pl.BlockSpec(memory_space=pl.ANY),
        out_shape=jax.ShapeDtypeStruct((H, C, W), bf16),
        scratch_shapes=[pltpu.VMEM((XF0 + 16 + NS * 12 + 1, C, 128), bf16), pltpu.VMEM((H + 2, C, 96), bf16),
                        pltpu.VMEM((H, C, 128), bf16), pltpu.VMEM((H, C, 96), bf16),
                        pltpu.VMEM((3, 3, C, C), bf16),
                        pltpu.VMEM((6, 2, C, 128), bf16), pltpu.VMEM((192, 128), bf16),
                        pltpu.VMEM((NS, 2, 6, 96, 128), u32),
                        pltpu.VMEM((NS, 2, 96, 128), u32),
                        pltpu.SemaphoreType.DMA((len(chunks) + 1,)), pltpu.SemaphoreType.DMA(())],
        compiler_params=pltpu.CompilerParams(vmem_limit_bytes=100 * 1024 * 1024),
    )(xt, w)
    return jnp.transpose(yt, (0, 2, 1))[None]


@jax.jit
def pallas_standalone__fft_conv__vision_kernel(x: jax.Array, w: jax.Array):
    return conv(x, w)
```

```python
import jax
import jax.numpy as jnp
from jax import lax
import jax.experimental.pallas as pl
import jax.experimental.pallas.tpu as pltpu

H = W = 224
C = 96
PA, PB = 2.0 / 3.0, 1.5
F32, BF16, U32 = jnp.float32, jnp.bfloat16, jnp.uint32

NT = H // 4
NS = 4
RING = 16
XF0 = H + 2
D0 = XF0 + RING
DUM = D0 + 12 * NS
MC = 48
NPART = 2 * (C // MC)
NROUND = 4 * NPART

SEGS = ((8, 1), (8, 6))
CHUNKS = ((0, 4), (4, 8), (8, 12), (12, 20), (20, 40), (40, 72), (72, 136), (136, 224))
T_AT = (0, 1, 3, 4, 5, 7, 8, 9, 11, 12, 13, 15)
R_AT = tuple(range(12))
F_AT = (0, 1, 2, 3)
F_DELAY = 3
J_ORDER = (1, 2, 3, 4, 0, 5)
OUT_START, OUT_GRAN, OUT_TAIL = 23, 4, 4


def _out_schedule():
    sched = {OUT_START: (0, OUT_START + 1)}
    s = OUT_START
    while s < NT - 1:
        g = OUT_GRAN if s + OUT_GRAN <= NT - 1 - OUT_TAIL else 1
        sched[s + g] = (s + 1, g)
        s += g
    return sched


def _kernel(x_hbm, w_hbm, y_hbm, big, xb1, yb0, yb1, wraw, u_ref, ul_ref, su, ltu,
            in_sems, out_sem):
    a, b = PA, PB
    a2, b2 = a * a, b * b

    def in_copies(k):
        lo, hi = CHUNKS[k]
        spans = ([(H - 2, 0, 2)] if k == 0 else []) + [(lo, lo + 2, hi - lo)]
        cps = []
        for src, dst, n in spans:
            cps.append(pltpu.make_async_copy(
                x_hbm.at[pl.ds(src, n), :, pl.ds(128, 96)], xb1.at[pl.ds(dst, n)], in_sems.at[k]))
            cps.append(pltpu.make_async_copy(
                x_hbm.at[pl.ds(src, n), :, pl.ds(0, 128)], big.at[pl.ds(dst, n)], in_sems.at[k]))
        return cps

    def wait_chunk(k):
        for cp in in_copies(k):
            cp.wait()

    def out_copy(n, lo, cnt):
        if n == 0:
            return pltpu.make_async_copy(
                yb0.at[pl.ds(lo, cnt)], y_hbm.at[pl.ds(lo, cnt), :, pl.ds(0, 128)], out_sem)
        return pltpu.make_async_copy(
            yb1.at[pl.ds(lo, cnt)], y_hbm.at[pl.ds(lo, cnt), :, pl.ds(128, 96)], out_sem)

    w_copy = pltpu.make_async_copy(w_hbm, wraw, in_sems.at[len(CHUNKS)])
    w_copy.start()
    for k in range(len(CHUNKS)):
        for cp in in_copies(k):
            cp.start()

    lane = lax.broadcasted_iota(jnp.int32, (8, 128), 1)
    m126 = lane >= 126
    m127 = lane >= 127
    zero = jnp.min(lane)

    bigu = big.bitcast(U32)
    xb1u = xb1.bitcast(U32)
    uu = u_ref.bitcast(U32)
    ulu = ul_ref.bitcast(U32)

    def weight_prep():
        eye = (lax.broadcasted_iota(jnp.int32, (C, C), 0)
               == lax.broadcasted_iota(jnp.int32, (C, C), 1)).astype(BF16)

        def tr_mxu(m):
            return lax.dot_general(eye, m.astype(BF16), (((1,), (1,)), ((), ())),
                                   preferred_element_type=F32).astype(BF16)

        def tr_xlu(m):
            return m.T.astype(BF16)

        def ktile(r, half):
            if half == 0:
                parts = [wraw[2 - r, 1, :, :], wraw[2 - r, 2, 0:32, :]]
            else:
                parts = [wraw[2 - r, 2, 32:96, :], wraw[2 - r, 0, 0:64, :]]
            return jnp.concatenate(parts, axis=0).astype(F32)

        g = [[ktile(r, half) for r in range(3)] for half in range(2)]
        fa = 1.0 / (2.0 * a2 * (a2 - b2))
        fb = 1.0 / (2.0 * b2 * (b2 - a2))
        for j, p, f in ((1, a, fa), (3, b, fb)):
            for half in range(2):
                g0, g1, g2 = g[half]
                ev = g0 * f + g2 * (f * p * p)
                od = g1 * (f * p)
                u_ref[j, half] = tr_mxu(ev + od)
                u_ref[j + 1, half] = tr_mxu(ev - od)
        for half in range(2):
            u_ref[0, half] = tr_xlu(g[half][0])
            u_ref[5, half] = tr_xlu(g[half][2])
        z = jnp.zeros((32, C), BF16)
        t0, t1, t2 = [wraw[2 - r, 0, 64:96, :] for r in range(3)]
        ul_ref[0:96, :] = tr_xlu(jnp.concatenate([t0, t1, t2, z], axis=0).astype(F32))
        ul_ref[96:192, :] = tr_xlu(jnp.concatenate([z, t0, t1, t2], axis=0).astype(F32))

    def fix_val(row):
        v = xb1u[row]
        return jnp.concatenate([v, v[:, 64:96]], axis=1)

    def dslab(slot, n, j):
        return D0 + (slot * 2 + n) * 6 + j

    def trans(tile, slot, vr, n, z):
        if n == 0:
            idx = [tile * 4 + k for k in range(6)]
        else:
            idx = [z + (XF0 + (slot * 4 + k) % RING) for k in range(6)]
        rows = pl.ds(vr * 16, 16)
        d = [big[idx[k], rows, :].astype(F32) for k in range(6)]
        if vr >= 4:
            for k in range(6):
                ltu[slot, n, pl.ds(k * 16 + (vr - 4) * 8, 8), :] = bigu[idx[k], pl.ds(vr * 8, 8), :]
        t = a2 * d[2]
        e1 = d[4] - b2 * d[2]
        o1 = a * d[3] - b * d[1]
        e2 = d[4] - t
        o2 = b * d[3] - a * d[1]
        out = [d[0] + e1 - t, e1 + o1, e1 - o1, e2 + o2, e2 - o2, d[1] - (a2 + b2) * d[3] + d[5]]
        for j in range(6):
            big[dslab(slot, n, j), rows, :] = out[j].astype(BF16)

    def rolls(slot, j, vrs, ns, z):
        for vr in vrs:
            v0 = bigu[z + dslab(slot, 0, j), pl.ds(vr * 8, 8), :]
            v1 = bigu[z + dslab(slot, 1, j), pl.ds(vr * 8, 8), :]
            if 0 in ns:
                su[slot, 0, j, pl.ds(vr * 8, 8), :] = pltpu.roll(jnp.where(m127, v1, v0), 1, 1)
                su[slot, 0, j, pl.ds(48 + vr * 8, 8), :] = pltpu.roll(jnp.where(m126, v1, v0), 2, 1)
            if 1 in ns:
                v1p = jnp.where(m126, v0, v1)
                su[slot, 1, j, pl.ds(vr * 8, 8), :] = pltpu.roll(v1p, 1, 1)
                su[slot, 1, j, pl.ds(48 + vr * 8, 8), :] = pltpu.roll(v1p, 2, 1)

    def dot(l, r):
        return jnp.dot(pltpu.bitcast(l, BF16), pltpu.bitcast(r, BF16), preferred_element_type=F32)

    def consume(tile, slot, part):
        r0 = tile * 4
        n, mc = divmod(part, C // MC)
        mr = pl.ds(mc * MC // 2, MC // 2)

        def mm(j):
            k1 = jnp.concatenate([su[slot, n, j, pl.ds(64, 32), :],
                                  bigu[dslab(slot, n, j), pl.ds(0, 32), :]], axis=0)
            return dot(uu[j, 0, mr, :], su[slot, n, j, pl.ds(0, 64), :]) + dot(uu[j, 1, mr, :], k1)

        def ll(p, h):
            return dot(ulu[pl.ds(48 * h + mc * MC // 2, MC // 2), :], ltu[slot, n, pl.ds(32 * p, 64), :])

        m1 = mm(1)
        m2 = mm(2)
        s12 = m1 + m2
        d12 = m1 - m2
        yield m1[0:8]
        m3 = mm(3)
        m4 = mm(4)
        s34 = m3 + m4
        d34 = m3 - m4
        y = [s12 + s34, a * d12 + b * d34, a2 * s12 + b2 * s34, (a2 * a) * d12 + (b2 * b) * d34]
        yield m3[0:8]
        m0 = mm(0)
        m5 = mm(5)
        y[0] = y[0] + m0
        y[3] = y[3] + m5
        yield m0[0:8]
        l0 = ll(0, 0)
        y = [y[0] + l0, y[1] + ll(0, 1), y[2] + ll(1, 0), y[3] + ll(1, 1)]
        for q in range(4):
            if n == 0:
                yb0[r0 + q, pl.ds(mc * MC, MC), :] = y[q].astype(BF16)
            else:
                yb1[r0 + q, pl.ds(mc * MC, MC), :] = y[q][:, :96].astype(BF16)
        yield l0[0:8]

    w_copy.wait()
    weight_prep()
    wait_chunk(0)
    for r in range(6):
        bigu[XF0 + r] = fix_val(r)
    for n in range(2):
        for vr in range(6):
            trans(0, 0, vr, n, 0)
    wait_chunk(1)
    for r in range(6, 10):
        bigu[XF0 + r] = fix_val(r)
    for j in J_ORDER:
        rolls(0, j, range(6), (0,), 0)
    for n in range(2):
        for vr in range(6):
            trans(1, 1, vr, n, 0)

    assert max(F_AT) + F_DELAY <= min(T_AT[6:])
    need_step = {k: next(s for s in range(NT) if 4 * (s + 2) + 4 > CHUNKS[k][0])
                 for k in range(2, len(CHUNKS))}
    osched = _out_schedule()

    def run_block(base, start, ntile, nrep, it):
        for t in range(ntile):
            cur = base + t
            statics = [start + i * ntile + t for i in range(nrep)]
            for k, s in need_step.items():
                if nrep == 1:
                    if s == statics[0]:
                        wait_chunk(k)
                elif t == 0 and start <= s < start + nrep * ntile:
                    pl.when(it == (s - start) // ntile)(lambda k=k: wait_chunk(k))
            s0 = (start + t) % NS
            s1 = (s0 + 1) % NS
            s2 = (s0 + 2) % NS
            if max(statics) + 2 < NT:
                n2 = cur + 2
            else:
                n2 = jnp.where(cur + 2 >= NT, cur + 2 - NT, cur + 2)

            def start_out(n):
                evs = [osched.get(s) for s in statics]
                rel = set(None if e is None else (s - e[0], e[1]) for s, e in zip(statics, evs))
                if len(rel) == 1:
                    (r,) = rel
                    if r is not None:
                        out_copy(n, (cur - r[0]) * 4, r[1] * 4).start()
                else:
                    for i, e in enumerate(evs):
                        if e is not None:
                            pl.when(it == i)(lambda e=e: out_copy(n, e[0] * 4, e[1] * 4).start())

            if statics == [0]:
                for j in J_ORDER:
                    rolls(0, j, range(6), (1,), 0)
            pending = []
            rnd = 0
            for part in range(NPART):
                gen = consume(cur, s0, part)
                for _ in range(4):
                    for due, ring, val in pending:
                        if due == rnd:
                            bigu[XF0 + ring] = val
                    for i in range(12):
                        if R_AT[i] == rnd:
                            rolls(s1, J_ORDER[i // 2], range(3 * (i % 2), 3 * (i % 2) + 3), (0, 1), zero)
                    for i in range(4):
                        if F_AT[i] == rnd:
                            pending.append((rnd + F_DELAY, (s2 * 4 + 2 + i) % RING, fix_val(n2 * 4 + 2 + i)))
                    for i in range(12):
                        if T_AT[i] == rnd:
                            trans(n2, s2, i % 6, i // 6, zero)
                    tick = pltpu.bitcast(next(gen), U32)
                    bigu[DUM, pl.ds(0, 8), :] = tick
                    if (rnd + 1) % NROUND in F_AT:
                        xb1u[H + 2, pl.ds(0, 8), :] = tick[:, :96]
                    rnd += 1
                if part == NPART // 2 - 1:
                    start_out(0)
                if part == NPART - 1:
                    start_out(1)

    start = 0
    for ntile, nrep in SEGS:
        if nrep == 1:
            run_block(zero + start, start, ntile, 1, None)
        else:
            assert ntile % NS == 0

            def body(it, carry, start=start, ntile=ntile, nrep=nrep):
                run_block(start + it * ntile, start, ntile, nrep, it)
                return carry

            lax.fori_loop(0, nrep, body, 0)
        start += ntile * nrep
    assert start == NT
    out_copy(0, 0, H).wait()
    out_copy(1, 0, H).wait()


@jax.jit
def pallas_standalone__fft_conv__vision_kernel(x: jax.Array, w: jax.Array):
    xt = jnp.transpose(x[0], (0, 2, 1))
    yt = pl.pallas_call(
        _kernel,
        in_specs=[pl.BlockSpec(memory_space=pl.ANY), pl.BlockSpec(memory_space=pl.ANY)],
        out_specs=pl.BlockSpec(memory_space=pl.ANY),
        out_shape=jax.ShapeDtypeStruct((H, C, W), BF16),
        scratch_shapes=[
            pltpu.VMEM((DUM + 1, C, 128), BF16),
            pltpu.VMEM((H + 3, C, 96), BF16),
            pltpu.VMEM((H, C, 128), BF16),
            pltpu.VMEM((H, C, 96), BF16),
            pltpu.VMEM((3, 3, C, C), BF16),
            pltpu.VMEM((6, 2, C, 128), BF16),
            pltpu.VMEM((192, 128), BF16),
            pltpu.VMEM((NS, 2, 6, 96, 128), U32),
            pltpu.VMEM((NS, 2, 96, 128), U32),
            pltpu.SemaphoreType.DMA((len(CHUNKS) + 1,)),
            pltpu.SemaphoreType.DMA(()),
        ],
        compiler_params=pltpu.CompilerParams(
            vmem_limit_bytes=64 * 1024 * 1024, disable_bounds_checks=True),
    )(xt, w)
    return jnp.transpose(yt, (0, 2, 1))[None]
```

```python
import jax
import jax.numpy as jnp
from jax import lax
import jax.experimental.pallas as pl
import jax.experimental.pallas.tpu as pltpu

H = W = 224
C = 96
PA, PB = 2.0 / 3.0, 1.5
F32, BF16, U32 = jnp.float32, jnp.bfloat16, jnp.uint32

NT = H // 4
NS = 4
RING = 16
D0 = H + 2
DUM = D0 + 12 * NS
MC = 48
NPART = 2 * (C // MC)
NROUND = 4 * NPART

SEGS = ((8, 1), (8, 6))
CHUNKS = ((0, 4), (4, 12), (12, 20), (20, 40), (40, 72), (72, 136), (136, 224))
T_AT = (0, 1, 2, 4, 5, 8, 9, 10, 12, 13, 14, 15)
R_AT = tuple(range(1, 13))
F_AT = (1, 3, 4, 4)
F_DELAY = 3
J_ORDER = (1, 2, 3, 4, 0, 5)
OUT_START, OUT_GRAN, OUT_TAIL = 23, 4, 4


def _out_schedule():
    sched = {OUT_START: (0, OUT_START + 1)}
    s = OUT_START
    while s < NT - 1:
        g = OUT_GRAN if s + OUT_GRAN <= NT - 1 - OUT_TAIL else 1
        sched[s + g] = (s + 1, g)
        s += g
    return sched


def _kernel(x_hbm, w_hbm, y_hbm, big, xb1, yb0, yb1, wraw, u_ref, ul_ref, su, lt, ring,
            in_sems, out_sem):
    a, b = PA, PB
    a2, b2 = a * a, b * b

    def in_copies(k):
        lo, hi = CHUNKS[k]
        spans = ([(H - 2, 0, 2)] if k == 0 else []) + [(lo, lo + 2, hi - lo)]
        cps = []
        for src, dst, n in spans:
            cps.append(pltpu.make_async_copy(
                x_hbm.at[pl.ds(src, n), :, pl.ds(128, 96)], xb1.at[pl.ds(dst, n)], in_sems.at[k]))
            cps.append(pltpu.make_async_copy(
                x_hbm.at[pl.ds(src, n), :, pl.ds(0, 128)], big.at[pl.ds(dst, n)], in_sems.at[k]))
        return cps

    def wait_chunk(k):
        for cp in in_copies(k):
            cp.wait()

    def out_copy(n, lo, cnt):
        if n == 0:
            return pltpu.make_async_copy(
                yb0.at[pl.ds(lo, cnt)], y_hbm.at[pl.ds(lo, cnt), :, pl.ds(0, 128)], out_sem)
        return pltpu.make_async_copy(
            yb1.at[pl.ds(lo, cnt)], y_hbm.at[pl.ds(lo, cnt), :, pl.ds(128, 96)], out_sem)

    w_copy = pltpu.make_async_copy(w_hbm, wraw, in_sems.at[len(CHUNKS)])
    w_copy.start()
    for k in range(len(CHUNKS)):
        for cp in in_copies(k):
            cp.start()

    lane = lax.broadcasted_iota(jnp.int32, (24, 128), 1)
    m126 = lane >= 126
    m127 = lane >= 127
    zero = jnp.min(lane[:8])

    def weight_prep():
        eye = (lax.broadcasted_iota(jnp.int32, (C, C), 0)
               == lax.broadcasted_iota(jnp.int32, (C, C), 1)).astype(BF16)

        def tr_mxu(m):
            return lax.dot_general(eye, m.astype(BF16), (((1,), (1,)), ((), ())),
                                   preferred_element_type=F32).astype(BF16)

        def tr_xlu(m):
            return m.T.astype(BF16)

        def pk(m):
            return pltpu.bitcast(m, U32)

        def ktile(r, half):
            if half == 0:
                parts = [wraw[2 - r, 1, :, :], wraw[2 - r, 2, 0:32, :]]
            else:
                parts = [wraw[2 - r, 2, 32:96, :], wraw[2 - r, 0, 0:64, :]]
            return jnp.concatenate(parts, axis=0).astype(F32)

        g = [[ktile(r, half) for r in range(3)] for half in range(2)]
        fa = 1.0 / (2.0 * a2 * (a2 - b2))
        fb = 1.0 / (2.0 * b2 * (b2 - a2))
        for j, p, f in ((1, a, fa), (3, b, fb)):
            for half in range(2):
                g0, g1, g2 = g[half]
                ev = g0 * f + g2 * (f * p * p)
                od = g1 * (f * p)
                u_ref[j, half] = pk(tr_mxu(ev + od))
                u_ref[j + 1, half] = pk(tr_mxu(ev - od))
        for half in range(2):
            u_ref[0, half] = pk(tr_xlu(g[half][0]))
            u_ref[5, half] = pk(tr_xlu(g[half][2]))
        z = jnp.zeros((32, C), BF16)
        t0, t1, t2 = [wraw[2 - r, 0, 64:96, :] for r in range(3)]
        ul_ref[0:48, :] = pk(tr_xlu(jnp.concatenate([t0, t1, t2, z], axis=0).astype(F32)))
        ul_ref[48:96, :] = pk(tr_xlu(jnp.concatenate([z, t0, t1, t2], axis=0).astype(F32)))

    def fix_val(row):
        v = pltpu.bitcast(xb1[row], U32)
        return jnp.concatenate([v, v[:, 64:96]], axis=1)

    def dslab(slot, n, j):
        return D0 + (slot * 2 + n) * 6 + j

    def trans(tile, slot, vr, n, z):
        rows = pl.ds(vr * 16, 16)
        if n == 0:
            raw = [big[tile * 4 + k, rows, :] for k in range(6)]
            if vr >= 4:
                for k in range(6):
                    lt[slot, pl.ds(k * 16 + (vr - 4) * 8, 8), :] = pltpu.bitcast(big[tile * 4 + k, rows, :], U32)
        else:
            raw = [pltpu.bitcast(ring[z + (slot * 4 + k) % RING, pl.ds(vr * 8, 8), :], BF16) for k in range(6)]
        d = [v.astype(F32) for v in raw]
        t = a2 * d[2]
        e1 = d[4] - b2 * d[2]
        o1 = a * d[3] - b * d[1]
        e2 = d[4] - t
        o2 = b * d[3] - a * d[1]
        out = [d[0] + e1 - t, e1 + o1, e1 - o1, e2 + o2, e2 - o2, d[1] - (a2 + b2) * d[3] + d[5]]
        for j in range(6):
            big[dslab(slot, n, j), rows, :] = out[j].astype(BF16)

    def rolls(slot, j, half, ns, z):
        v0 = pltpu.bitcast(big[z + dslab(slot, 0, j), pl.ds(half * 48, 48), :], U32)
        v1 = pltpu.bitcast(big[z + dslab(slot, 1, j), pl.ds(half * 48, 48), :], U32)
        n0 = 24 if half == 0 else 8
        if 0 in ns:
            su[slot, 0, j, pl.ds(half * 24, 24), :] = pltpu.roll(jnp.where(m127, v1, v0), 1, 1)
            su[slot, 0, j, pl.ds(48 + half * 24, 24), :] = pltpu.roll(jnp.where(m126, v1, v0), 2, 1)
            su[slot, 0, j, pl.ds(96 + half * 24, n0), :] = v0[:n0]
        if 1 in ns:
            v1p = jnp.where(m126, v0, v1)
            su[slot, 1, j, pl.ds(half * 24, 24), :] = pltpu.roll(v1p, 1, 1)
            su[slot, 1, j, pl.ds(48 + half * 24, 24), :] = pltpu.roll(v1p, 2, 1)
            su[slot, 1, j, pl.ds(96 + half * 24, n0), :] = v1[:n0]

    def dot(l, r):
        return jnp.dot(pltpu.bitcast(l, BF16), pltpu.bitcast(r, BF16), preferred_element_type=F32)

    def consume(tile, slot, part):
        r0 = tile * 4
        n, mc = divmod(part, C // MC)
        mr = pl.ds(mc * MC // 2, MC // 2)

        def mm(j):
            return (dot(u_ref[j, 0, mr, :], su[slot, n, j, pl.ds(0, 64), :])
                    + dot(u_ref[j, 1, mr, :], su[slot, n, j, pl.ds(64, 64), :]))

        def ll(p, h):
            if n == 0:
                rhs = lt[slot, pl.ds(32 * p, 64), :]
            else:
                rhs = jnp.concatenate(
                    [ring[(slot * 4 + 2 * p + k) % RING, pl.ds(32, 16), :] for k in range(4)], axis=0)
            return dot(ul_ref[pl.ds(48 * h + mc * MC // 2, MC // 2), :], rhs)

        m1 = mm(1)
        m2 = mm(2)
        s12 = m1 + m2
        d12 = m1 - m2
        yield m1[0:16]
        m3 = mm(3)
        m4 = mm(4)
        s34 = m3 + m4
        d34 = m3 - m4
        y = [s12 + s34, a * d12 + b * d34, a2 * s12 + b2 * s34, (a2 * a) * d12 + (b2 * b) * d34]
        yield m3[0:16]
        m0 = mm(0)
        m5 = mm(5)
        y[0] = y[0] + m0
        y[3] = y[3] + m5
        yield m0[0:16]
        l0 = ll(0, 0)
        y = [y[0] + l0, y[1] + ll(0, 1), y[2] + ll(1, 0), y[3] + ll(1, 1)]
        for q in range(4):
            if n == 0:
                yb0[r0 + q, pl.ds(mc * MC, MC), :] = y[q].astype(BF16)
            else:
                yb1[r0 + q, pl.ds(mc * MC, MC), :] = y[q][:, :96].astype(BF16)
        yield l0[0:16]

    w_copy.wait()
    weight_prep()
    wait_chunk(0)
    for r in range(6):
        ring[r] = fix_val(r)
    for n in range(2):
        for vr in range(6):
            trans(zero, 0, vr, n, 0)
    for j in J_ORDER:
        for half in range(2):
            rolls(0, j, half, (0,), 0)

    assert max(F_AT) + F_DELAY <= min(T_AT[6:])
    need_step = {k: next(s for s in range(NT) if 4 * (s + 2) + 4 > CHUNKS[k][0])
                 for k in range(1, len(CHUNKS))}
    osched = _out_schedule()

    def run_block(base, start, ntile, nrep, it):
        for t in range(ntile):
            cur = base + t
            statics = [start + i * ntile + t for i in range(nrep)]
            for k, s in need_step.items():
                if nrep == 1:
                    if s == statics[0]:
                        wait_chunk(k)
                elif t == 0 and start <= s < start + nrep * ntile:
                    pl.when(it == (s - start) // ntile)(lambda k=k: wait_chunk(k))
            s0 = (start + t) % NS
            s1 = (s0 + 1) % NS
            s2 = (s0 + 2) % NS
            if max(statics) + 2 < NT:
                n2 = cur + 2
            else:
                n2 = jnp.where(cur + 2 >= NT, cur + 2 - NT, cur + 2)

            def start_out(n):
                evs = [osched.get(s) for s in statics]
                rel = set(None if e is None else (s - e[0], e[1]) for s, e in zip(statics, evs))
                if len(rel) == 1:
                    (r,) = rel
                    if r is not None:
                        out_copy(n, (cur - r[0]) * 4, r[1] * 4).start()
                else:
                    for i, e in enumerate(evs):
                        if e is not None:
                            pl.when(it == i)(lambda e=e: out_copy(n, e[0] * 4, e[1] * 4).start())

            if statics == [0]:
                for r in range(6, 10):
                    ring[r] = fix_val(r)
                for j in J_ORDER:
                    for half in range(2):
                        rolls(0, j, half, (1,), 0)
                for n in range(2):
                    for vr in range(6):
                        trans(zero + 1, 1, vr, n, 0)
            pending = []
            rnd = 0
            for part in range(NPART):
                gen = consume(cur, s0, part)
                for _ in range(4):
                    for due, row, val in pending:
                        if due == rnd:
                            ring[row] = val
                    for i in range(12):
                        if R_AT[i] == rnd:
                            rolls(s1, J_ORDER[i // 2], i % 2, (0, 1), zero)
                    for i in range(4):
                        if F_AT[i] == rnd:
                            pending.append((rnd + F_DELAY, (s2 * 4 + 2 + i) % RING, fix_val(n2 * 4 + 2 + i)))
                    for i in range(12):
                        if T_AT[i] == rnd:
                            trans(n2, s2, i % 6, i // 6, zero)
                    tick = next(gen)
                    big[DUM, pl.ds(0, 16), :] = tick.astype(BF16)
                    if (rnd + 1) % NROUND in T_AT[6:]:
                        ring[RING, pl.ds(0, 8), :] = pltpu.bitcast(tick[0:8], U32)
                    if (rnd + 1) % NROUND in F_AT:
                        xb1[H + 2, pl.ds(0, 16), :] = tick[:, :96].astype(BF16)
                    rnd += 1
                if part == NPART // 2 - 1:
                    start_out(0)
                if part == NPART - 1:
                    start_out(1)

    start = 0
    for ntile, nrep in SEGS:
        if nrep == 1:
            run_block(zero + start, start, ntile, 1, None)
        else:
            assert ntile % NS == 0

            def body(it, carry, start=start, ntile=ntile, nrep=nrep):
                run_block(start + it * ntile, start, ntile, nrep, it)
                return carry

            lax.fori_loop(0, nrep, body, 0)
        start += ntile * nrep
    assert start == NT
    out_copy(0, 0, H).wait()
    out_copy(1, 0, H).wait()


@jax.jit
def pallas_standalone__fft_conv__vision_kernel(x: jax.Array, w: jax.Array):
    xt = jnp.transpose(x.reshape(H, W, C), (0, 2, 1))
    yt = pl.pallas_call(
        _kernel,
        in_specs=[pl.BlockSpec(memory_space=pl.ANY), pl.BlockSpec(memory_space=pl.ANY)],
        out_specs=pl.BlockSpec(memory_space=pl.ANY),
        out_shape=jax.ShapeDtypeStruct((H, C, W), BF16),
        scratch_shapes=[
            pltpu.VMEM((DUM + 1, C, 128), BF16),
            pltpu.VMEM((H + 3, C, 96), BF16),
            pltpu.VMEM((H, C, 128), BF16),
            pltpu.VMEM((H, C, 96), BF16),
            pltpu.VMEM((3, 3, C, C), BF16),
            pltpu.VMEM((6, 2, 48, 128), U32),
            pltpu.VMEM((96, 128), U32),
            pltpu.VMEM((NS, 2, 6, 128, 128), U32),
            pltpu.VMEM((NS, 96, 128), U32),
            pltpu.VMEM((RING + 1, 48, 128), U32),
            pltpu.SemaphoreType.DMA((len(CHUNKS) + 1,)),
            pltpu.SemaphoreType.DMA(()),
        ],
        compiler_params=pltpu.CompilerParams(vmem_limit_bytes=64 * 1024 * 1024),
    )(xt, w)
    return jnp.transpose(yt, (0, 2, 1)).reshape(1, H, W, C)
```
